```python
import os as _os
_os.environ.setdefault("JAX_PLATFORMS", "cpu")
import jax
import jax.numpy as jnp

def _softmax(x, axis=-1):
    return jax.nn.softmax(x, axis=axis)
def _gelu(x):
    return jax.nn.gelu(x, approximate=True)
def _silu(x):
    return jax.nn.silu(x)
def _sigmoid(x):
    return jax.nn.sigmoid(x)
def _layernorm(x, axis=-1, eps=1e-5):
    m = jnp.mean(x, axis=axis, keepdims=True)
    v = jnp.var(x, axis=axis, keepdims=True)
    return (x - m) / jnp.sqrt(v + eps)
def _scatter_add(tgt, idx, src, axis=0):
    return tgt.at[idx].add(src)
def _segment_sum(src, seg, n):
    return jax.ops.segment_sum(src, seg, n)
class _Rng:
    def __init__(self, key):
        self._k = key
    def _next(self):
        self._k, sub = jax.random.split(self._k)
        return sub
    def normal(self, shape):
        return jax.random.normal(self._next(), shape, dtype=jnp.bfloat16)
    def randint(self, lo, hi, shape):
        return jax.random.randint(self._next(), shape, lo, hi, dtype=jnp.int32)
    def uniform(self, shape, lo=0.0, hi=1.0):
        return jax.random.uniform(self._next(), shape, jnp.bfloat16, lo, hi)
    def permutation(self, n):
        return jax.random.permutation(self._next(), n)


kernel_name = 'sequential_preLN__linear_attn_block__glu_gated_reglu__prompt'

def setup_inputs():
    _rng = _Rng(jax.random.key(int.from_bytes(__import__("os").urandom(4), "little")))
    _w = (lambda a: (lambda t: t.astype(jnp.bfloat16) if jnp.issubdtype(t.dtype, jnp.floating) else t)(jnp.asarray(a)))
    def _A_setup():
        B, S, D = 1, 2048, 640
        return {
            "x": _w((lambda *s: _rng.normal(s) * 0.05)(B, S, D)),
            "wqkv": _w((lambda *s: _rng.normal(s) * 0.05)(D, 3 * D)),
            "wo": _w((lambda *s: _rng.normal(s) * 0.05)(D, D)),
        }
    _A_in = _A_setup()

    def _B_setup():
        B, S, D, F = 1, 2048, 640, 1536
        return {
            "x": _w((lambda *s: _rng.normal(s) * 0.05)(B, S, D)),
            "W_gate": _w((lambda *s: _rng.normal(s) * 0.05)(D, F) * (2.0 / D) ** 0.5),
            "W_up": _w((lambda *s: _rng.normal(s) * 0.05)(D, F) * (2.0 / D) ** 0.5),
            "W_down": _w((lambda *s: _rng.normal(s) * 0.05)(F, D) * (1.0 / F) ** 0.5),
        }
    _B_in = _B_setup()

    return {
        "A_x": _A_in["x"],
        "A_wqkv": _A_in["wqkv"],
        "A_wo": _A_in["wo"],
        "B_x": _B_in["x"],
        "B_W_gate": _B_in["W_gate"],
        "B_W_up": _B_in["W_up"],
        "B_W_down": _B_in["W_down"],
    }

def reference(A_x, A_wqkv, A_wo, B_x, B_W_gate, B_W_up, B_W_down):
    def _A_ref(x, wqkv, wo):
        B, S, D = x.shape
        H = 32; Dh = D // H
        qkv = (lambda x, *d: x.transpose(*d))((x @ wqkv).reshape(B, S, 3, H, Dh), 2, 0, 3, 1, 4)
        q, k, v = qkv[0], qkv[1], qkv[2]
        phi = lambda t: jnp.where(t > 0, t + 1, jnp.exp(t)) + 1e-6
        pq, pk = phi(q), phi(k)
        kv = jnp.einsum("bhsd,bhse->bhde", pk, v)
        z = jnp.einsum("bhsd->bhd", pk)
        num = jnp.einsum("bhqd,bhde->bhqe", pq, kv)
        den = jnp.einsum("bhqd,bhd->bhq", pq, z)[..., None] + 1e-6
        o = num / den
        return (lambda x, *d: x.transpose(*d))(o, 0, 2, 1, 3).reshape(B, S, D) @ wo

    def _B_ref(x, W_gate, W_up, W_down):
        gate = jnp.einsum("bsd,df->bsf", x, W_gate)
        up = jnp.einsum("bsd,df->bsf", x, W_up)
        gate = gate * (lambda x, dt: x.astype(dt))(gate > 0, gate.dtype)
        h = gate * up
        return jnp.einsum("bsf,fd->bsd", h, W_down)

    x = A_x
    h = x + _A_ref(_layernorm(x, axis=-1), A_wqkv, A_wo)
    h2 = h + _B_ref(_layernorm(h, axis=-1), B_W_gate, B_W_up, B_W_down)
    return h2
```

```python
import jax
import jax.numpy as jnp
from jax import lax
import jax.experimental.pallas as pl
import jax.experimental.pallas.tpu as pltpu

S, D, F, H = 2048, 640, 1536, 32
DH = D // H
T1 = 512
T2 = 256
NT = D // 128
LNC = 32
BF = jnp.bfloat16
F32 = jnp.float32


def _ln(x):
    m = jnp.mean(x, axis=-1, keepdims=True)
    xc = x - m
    v = jnp.mean(xc * xc, axis=-1, keepdims=True)
    return xc * lax.rsqrt(v + 1e-5)


def _ln_rows(ref, r0, n, c=LNC):
    outs = []
    for k in range(n // c):
        outs.append(_ln(ref[pl.ds(r0 + k * c, c), :].astype(F32)).astype(BF))
    return jnp.concatenate(outs, axis=0)


def _phi(t):
    return jnp.where(t > 0, t + 1.0, jnp.exp(t)) + 1e-6


def _dot(a, b):
    return jnp.dot(a, b, preferred_element_type=F32)


def _dot_nt(a, b):
    return lax.dot_general(a, b, (((1,), (1,)), ((), ())), preferred_element_type=F32)


def _kernel(x_hbm, wqkv_hbm, wo_hbm, wg_hbm, wu_hbm, wd_hbm, o_hbm,
            x_v, xn_v, wq_v, wk_v, wv_v, wkT_v, wqT_v, wo_v, wg_v, wu_v, wd_v, o_v, h_v,
            g_v, z_v, m_v, slab_v, zrow_v, sems, osems):
    n1 = S // T1
    n2 = S // T2

    def rows(i, t):
        if isinstance(i, int):
            return pl.ds(i * t, t)
        return pl.ds(pl.multiple_of(i * t, t), t)

    def xcopy(i):
        return pltpu.make_async_copy(x_hbm.at[rows(i, T1)], x_v.at[rows(i, T1)], sems.at[i])

    def ocopy(i):
        return pltpu.make_async_copy(o_v.at[rows(i, T2)], o_hbm.at[rows(i, T2)], osems.at[i])
    wk_c = pltpu.make_async_copy(wqkv_hbm.at[:, pl.ds(D, D)], wk_v, sems.at[n1])
    wv_c = pltpu.make_async_copy(wqkv_hbm.at[:, pl.ds(2 * D, D)], wv_v, sems.at[n1 + 1])
    wq_c = pltpu.make_async_copy(wqkv_hbm.at[:, pl.ds(0, D)], wq_v, sems.at[n1 + 2])
    wo_c = pltpu.make_async_copy(wo_hbm, wo_v, sems.at[n1 + 3])
    wg_c = pltpu.make_async_copy(wg_hbm, wg_v, sems.at[n1 + 4])
    wu_c = pltpu.make_async_copy(wu_hbm, wu_v, sems.at[n1 + 5])
    wd_c = pltpu.make_async_copy(wd_hbm, wd_v, sems.at[n1 + 6])
    c0 = 128
    x0a = pltpu.make_async_copy(x_hbm.at[pl.ds(0, c0)], x_v.at[pl.ds(0, c0)], sems.at[n1 + 7])
    x0b = pltpu.make_async_copy(x_hbm.at[pl.ds(c0, T1 - c0)], x_v.at[pl.ds(c0, T1 - c0)], sems.at[0])
    x0a.start()
    wk_c.start()
    x0b.start()
    xcopy(1).start()

    def ln1(i):
        xcopy(i).wait()
        xn_v[rows(i, T1), :] = _ln_rows(x_v, i * T1, T1)

    def kg(i, first=False, last=False, kT=None):
        xn = xn_v[rows(i, T1), :]
        if kT is None:
            kT = _dot_nt(wkT_v[...], xn)
        pkT = _phi(kT)
        zz = pkT[:, 0:128]
        for t in range(1, T1 // 128):
            zz = zz + pkT[:, t * 128:(t + 1) * 128]
        gg = _dot(pkT.astype(BF), xn)
        if last:
            z_v[...] += zz
            return (g_v[...] + gg).astype(BF)
        if first:
            z_v[...] = zz
            g_v[...] = gg
        else:
            z_v[...] += zz
            g_v[...] += gg

    for i in range(2, n1):
        xcopy(i).start()
    wq_c.start(); wv_c.start(); wo_c.start(); wg_c.start(); wu_c.start(); wd_c.start()
    x0a.wait()
    ks = []
    for c in range(T1 // c0):
        xc = _ln_rows(x_v, c * c0, c0)
        xn_v[pl.ds(c * c0, c0), :] = xc
        if c == 0:
            wk_c.wait()
            x0b.wait()
        if c == 2:
            xcopy(1).wait()
        ks.append(_dot(xc, wk_v[...]))
    kg(0, first=True, kT=jnp.concatenate([k.T for k in ks], axis=1))
    wkT_v[...] = wk_v[...].T
    xn_v[rows(1, T1), :] = _ln_rows(x_v, T1, T1)

    def p1(i, c):
        xcopy(i + 1).wait()
        kg(i)
        xn_v[rows(i + 1, T1), :] = _ln_rows(x_v, (i + 1) * T1, T1)
        return c
    lax.fori_loop(1, n1 - 1, p1, 0)

    def permute_rows(dst_ref):
        for j in range(DH):
            for ct in range(NT):
                dst_ref[j * H:(j + 1) * H, ct * 128:(ct + 1) * 128] = (
                    slab_v[ct, pl.ds(j, H, stride=DH), :].astype(BF))

    wq_c.wait(); wv_c.wait(); wo_c.wait()
    for ct in range(NT):
        slab_v[ct] = wq_v[ct * 128:(ct + 1) * 128, :].astype(F32).T
    permute_rows(wqT_v)
    gb = kg(n1 - 1, last=True)

    def stage_a(i):
        pq = _phi(_dot_nt(xn_v[rows(i, T2), :], wqT_v[...]))
        return pq

    def stage_a2(pq):
        w = pq * zrow_v[0:1, :]
        s = w[:, 0:128]
        for t in range(1, NT):
            s = s + w[:, t * 128:(t + 1) * 128]
        s = s + pltpu.roll(s, 64, 1)
        s = s + pltpu.roll(s, 32, 1)
        rr = 1.0 / (s + 1e-6)
        return jnp.concatenate([pq[:, t * 128:(t + 1) * 128] * rr for t in range(NT)], axis=1).astype(BF)

    def stage_b(i, pqn):
        h = x_v[rows(i, T2), :].astype(F32) + _dot(pqn, m_v[...])
        return h

    def stage_b2(i, h):
        h_v[rows(i, T2), :] = h
        xn_v[rows(i, T2), :] = _ln(h).astype(BF)

    def stage_c1(i):
        return _dot(xn_v[rows(i, T2), :], wg_v[...])

    def stage_c2(i):
        return _dot(xn_v[rows(i, T2), :], wu_v[...])

    def stage_c3(i, g, u):
        a = (jnp.maximum(g, 0.0) * u).astype(BF)
        o = h_v[rows(i, T2), :] + _dot(a, wd_v[...])
        o_v[rows(i, T2), :] = o.astype(BF)
        ocopy(i).start()

    lo = [max(j - 1, 0) for j in range(NT)]
    hi = [min(j + 2, NT) for j in range(NT)]
    kvs = []
    for j in range(NT):
        kv = _dot(gb[lo[j] * 128:hi[j] * 128, :], wv_v[:, j * 128:(j + 1) * 128])
        shp = kv.shape
        rh = ((lax.broadcasted_iota(jnp.int32, shp, 0) + lo[j] * 128) * 3277) >> 16
        ch = ((lax.broadcasted_iota(jnp.int32, shp, 1) + j * 128) * 3277) >> 16
        kvs.append(jnp.where(rh == ch, kv, 0.0).astype(BF))
    zp = jnp.concatenate([z_v[pl.ds(j, H, stride=DH), :] for j in range(DH)], axis=0)
    zrow_v[...] = jnp.broadcast_to(jnp.sum(zp.T, axis=0, keepdims=True), zrow_v.shape)
    parts = [_dot(kvs[j], wo_v[j * 128:(j + 1) * 128, :]) for j in range(NT)]
    for i in range(NT):
        mt = None
        for j in range(NT):
            if lo[j] <= i < hi[j]:
                p = parts[j][(i - lo[j]) * 128:(i - lo[j] + 1) * 128, :]
                mt = p if mt is None else mt + p
        for ct in range(NT):
            slab_v[ct, i * 128:(i + 1) * 128, :] = mt[:, ct * 128:(ct + 1) * 128]
    permute_rows(m_v)
    wg_c.wait(); wu_c.wait(); wd_c.wait()

    def p2(k, c):
        a, b = 2 * k, 2 * k + 1
        pqa = stage_a(a)
        pqb = stage_a(b)
        ha = stage_b(a, stage_a2(pqa))
        hb = stage_b(b, stage_a2(pqb))
        hna = _ln(ha).astype(BF)
        hnb = _ln(hb).astype(BF)
        for (t, h, hn) in ((a, ha, hna), (b, hb, hnb)):
            g = _dot(hn, wg_v[...])
            u = _dot(hn, wu_v[...])
            act = (jnp.maximum(g, 0.0) * u).astype(BF)
            o = h + _dot(act, wd_v[...])
            o_v[rows(t, T2), :] = o.astype(BF)
            ocopy(t).start()
        return c
    lax.fori_loop(0, n2 // 2, p2, 0)

    def fin(i, c):
        ocopy(i).wait()
        return c
    lax.fori_loop(0, n2, fin, 0)


@jax.jit
def pallas_sequential_preLN__linear_attn_block__glu_gated_reglu__prompt_kernel(A_x, A_wqkv, A_wo, B_x, B_W_gate, B_W_up, B_W_down):
    del B_x
    x = A_x.reshape(S, D)
    n1 = S // T1
    n2 = S // T2
    anyspec = pl.BlockSpec(memory_space=pl.ANY)
    out = pl.pallas_call(
        _kernel,
        out_shape=jax.ShapeDtypeStruct((S, D), BF),
        in_specs=[anyspec] * 6,
        out_specs=anyspec,
        scratch_shapes=[
            pltpu.VMEM((S, D), BF), pltpu.VMEM((S, D), BF),
            pltpu.VMEM((D, D), BF), pltpu.VMEM((D, D), BF), pltpu.VMEM((D, D), BF), pltpu.VMEM((D, D), BF), pltpu.VMEM((D, D), BF),
            pltpu.VMEM((D, D), BF), pltpu.VMEM((D, F), BF), pltpu.VMEM((D, F), BF), pltpu.VMEM((F, D), BF),
            pltpu.VMEM((S, D), BF), pltpu.VMEM((S, D), F32),
            pltpu.VMEM((D, D), F32), pltpu.VMEM((D, 128), F32), pltpu.VMEM((D, D), BF),
            pltpu.VMEM((NT, D, 128), F32), pltpu.VMEM((8, D), F32),
            pltpu.SemaphoreType.DMA((n1 + 8,)), pltpu.SemaphoreType.DMA((n2,)),
        ],
        compiler_params=pltpu.CompilerParams(vmem_limit_bytes=100 * 1024 * 1024),
    )(x, A_wqkv, A_wo, B_W_gate, B_W_up, B_W_down)
    return out.reshape(1, S, D)
```

```python
import jax
import jax.numpy as jnp
from jax import lax
import jax.experimental.pallas as pl
import jax.experimental.pallas.tpu as pltpu

S, D, F, H = 2048, 640, 1536, 32
DH = D // H
T1 = 512
T2 = 256
NT = D // 128
LNC = 32
BF = jnp.bfloat16
F32 = jnp.float32


def _ln(x):
    m = jnp.mean(x, axis=-1, keepdims=True)
    xc = x - m
    v = jnp.mean(xc * xc, axis=-1, keepdims=True)
    return xc * lax.rsqrt(v + 1e-5)


def _ln_rows(ref, r0, n, c=LNC):
    outs = []
    for k in range(n // c):
        outs.append(_ln(ref[pl.ds(r0 + k * c, c), :].astype(F32)).astype(BF))
    return jnp.concatenate(outs, axis=0)


def _phi(t):
    return jnp.where(t > 0, t + 1.0, jnp.exp(t)) + 1e-6


def _dot(a, b):
    return jnp.dot(a, b, preferred_element_type=F32)


def _dot_nt(a, b):
    return lax.dot_general(a, b, (((1,), (1,)), ((), ())), preferred_element_type=F32)


def _kernel(x_hbm, wqkv_hbm, wo_hbm, wg_hbm, wu_hbm, wd_hbm, o_hbm,
            x_v, xn_v, wq_v, wk_v, wv_v, wkT_v, wqT_v, wo_v, wg_v, wu_v, wd_v, o_v, h_v,
            g_v, z_v, m_v, slab_v, zrow_v, sems, osems):
    n1 = S // T1
    n2 = S // T2

    def rows(i, t):
        if isinstance(i, int):
            return pl.ds(i * t, t)
        return pl.ds(pl.multiple_of(i * t, t), t)

    def xcopy(i):
        return pltpu.make_async_copy(x_hbm.at[rows(i, T1)], x_v.at[rows(i, T1)], sems.at[i])

    def ocopy(i):
        return pltpu.make_async_copy(o_v.at[rows(i, T2)], o_hbm.at[rows(i, T2)], osems.at[i])
    NA = 256
    wk_c = pltpu.make_async_copy(wqkv_hbm.at[:, pl.ds(D, NA)], wk_v.at[:, pl.ds(0, NA)], sems.at[n1])
    wk_d = pltpu.make_async_copy(wqkv_hbm.at[:, pl.ds(D + NA, D - NA)], wk_v.at[:, pl.ds(NA, D - NA)], sems.at[n1 + 8])
    wv_c = pltpu.make_async_copy(wqkv_hbm.at[:, pl.ds(2 * D, D)], wv_v, sems.at[n1 + 1])
    wq_c = pltpu.make_async_copy(wqkv_hbm.at[:, pl.ds(0, D)], wq_v, sems.at[n1 + 2])
    wo_c = pltpu.make_async_copy(wo_hbm, wo_v, sems.at[n1 + 3])
    wg_c = pltpu.make_async_copy(wg_hbm, wg_v, sems.at[n1 + 4])
    wu_c = pltpu.make_async_copy(wu_hbm, wu_v, sems.at[n1 + 5])
    wd_c = pltpu.make_async_copy(wd_hbm, wd_v, sems.at[n1 + 6])
    c0 = 128
    x0a = pltpu.make_async_copy(x_hbm.at[pl.ds(0, c0)], x_v.at[pl.ds(0, c0)], sems.at[n1 + 7])
    x0b = pltpu.make_async_copy(x_hbm.at[pl.ds(c0, T1 - c0)], x_v.at[pl.ds(c0, T1 - c0)], sems.at[0])
    x0a.start()
    wk_c.start()
    x0b.start()
    wk_d.start()
    xcopy(1).start()

    def ln1(i):
        xcopy(i).wait()
        xn_v[rows(i, T1), :] = _ln_rows(x_v, i * T1, T1)

    def kg(i, first=False, last=False, kT=None):
        xn = xn_v[rows(i, T1), :]
        if kT is None:
            kT = _dot_nt(wkT_v[...], xn)
        pkT = _phi(kT)
        zz = pkT[:, 0:128]
        for t in range(1, T1 // 128):
            zz = zz + pkT[:, t * 128:(t + 1) * 128]
        gg = _dot(pkT.astype(BF), xn)
        if last:
            z_v[...] += zz
            return (g_v[...] + gg).astype(BF)
        if first:
            z_v[...] = zz
            g_v[...] = gg
        else:
            z_v[...] += zz
            g_v[...] += gg

    for i in range(2, n1):
        xcopy(i).start()
    wq_c.start(); wv_c.start(); wo_c.start(); wg_c.start(); wu_c.start(); wd_c.start()
    x0a.wait()
    xs, ka, kb = [], [], []
    for c in range(T1 // c0):
        if c == 1:
            x0b.wait()
        xc = _ln_rows(x_v, c * c0, c0)
        xn_v[pl.ds(c * c0, c0), :] = xc
        xs.append(xc)
        if c == 0:
            wk_c.wait()
        ka.append(_dot(xc, wk_v[:, 0:NA]))
    wk_d.wait()
    xcopy(1).wait()
    for c in range(T1 // c0):
        kb.append(_dot(xn_v[pl.ds(c * c0, c0), :], wk_v[:, NA:D]))
    kg(0, first=True, kT=jnp.concatenate(
        [jnp.concatenate([a, b], axis=1).T for a, b in zip(ka, kb)], axis=1))
    wkT_v[...] = wk_v[...].T
    xn_v[rows(1, T1), :] = _ln_rows(x_v, T1, T1)

    def p1(i, c):
        xcopy(i + 1).wait()
        kg(i)
        xn_v[rows(i + 1, T1), :] = _ln_rows(x_v, (i + 1) * T1, T1)
        return c
    lax.fori_loop(1, n1 - 1, p1, 0)

    def permute_rows(dst_ref):
        for j in range(DH):
            for ct in range(NT):
                dst_ref[j * H:(j + 1) * H, ct * 128:(ct + 1) * 128] = (
                    slab_v[ct, pl.ds(j, H, stride=DH), :].astype(BF))

    wq_c.wait(); wv_c.wait(); wo_c.wait()
    for ct in range(NT):
        slab_v[ct] = wq_v[ct * 128:(ct + 1) * 128, :].astype(F32).T
    permute_rows(wqT_v)
    gb = kg(n1 - 1, last=True)

    def stage_a(i):
        pq = _phi(_dot_nt(xn_v[rows(i, T2), :], wqT_v[...]))
        return pq

    def stage_a2(pq):
        w = pq * zrow_v[0:1, :]
        s = w[:, 0:128]
        for t in range(1, NT):
            s = s + w[:, t * 128:(t + 1) * 128]
        s = s + pltpu.roll(s, 64, 1)
        s = s + pltpu.roll(s, 32, 1)
        rr = 1.0 / (s + 1e-6)
        return jnp.concatenate([pq[:, t * 128:(t + 1) * 128] * rr for t in range(NT)], axis=1).astype(BF)

    def stage_b(i, pqn):
        h = x_v[rows(i, T2), :].astype(F32) + _dot(pqn, m_v[...])
        return h

    def stage_b2(i, h):
        h_v[rows(i, T2), :] = h
        xn_v[rows(i, T2), :] = _ln(h).astype(BF)

    def stage_c1(i):
        return _dot(xn_v[rows(i, T2), :], wg_v[...])

    def stage_c2(i):
        return _dot(xn_v[rows(i, T2), :], wu_v[...])

    def stage_c3(i, g, u):
        a = (jnp.maximum(g, 0.0) * u).astype(BF)
        o = h_v[rows(i, T2), :] + _dot(a, wd_v[...])
        o_v[rows(i, T2), :] = o.astype(BF)
        ocopy(i).start()

    lo = [max(j - 1, 0) for j in range(NT)]
    hi = [min(j + 2, NT) for j in range(NT)]
    kvs = []
    for j in range(NT):
        kv = _dot(gb[lo[j] * 128:hi[j] * 128, :], wv_v[:, j * 128:(j + 1) * 128])
        shp = kv.shape
        rh = ((lax.broadcasted_iota(jnp.int32, shp, 0) + lo[j] * 128) * 3277) >> 16
        ch = ((lax.broadcasted_iota(jnp.int32, shp, 1) + j * 128) * 3277) >> 16
        kvs.append(jnp.where(rh == ch, kv, 0.0).astype(BF))
    zp = jnp.concatenate([z_v[pl.ds(j, H, stride=DH), :] for j in range(DH)], axis=0)
    zrow_v[...] = jnp.broadcast_to(jnp.sum(zp.T, axis=0, keepdims=True), zrow_v.shape)
    parts = [_dot(kvs[j], wo_v[j * 128:(j + 1) * 128, :]) for j in range(NT)]
    for i in range(NT):
        mt = None
        for j in range(NT):
            if lo[j] <= i < hi[j]:
                p = parts[j][(i - lo[j]) * 128:(i - lo[j] + 1) * 128, :]
                mt = p if mt is None else mt + p
        for ct in range(NT):
            slab_v[ct, i * 128:(i + 1) * 128, :] = mt[:, ct * 128:(ct + 1) * 128]
    permute_rows(m_v)
    wg_c.wait(); wu_c.wait(); wd_c.wait()

    def p2(k, c):
        a, b = 2 * k, 2 * k + 1
        pqa = stage_a(a)
        pqb = stage_a(b)
        ha = stage_b(a, stage_a2(pqa))
        hb = stage_b(b, stage_a2(pqb))
        hna = _ln(ha).astype(BF)
        hnb = _ln(hb).astype(BF)
        for (t, h, hn) in ((a, ha, hna), (b, hb, hnb)):
            g = _dot(hn, wg_v[...])
            u = _dot(hn, wu_v[...])
            act = (jnp.maximum(g, 0.0) * u).astype(BF)
            o = h + _dot(act, wd_v[...])
            o_v[rows(t, T2), :] = o.astype(BF)
            ocopy(t).start()
        return c
    lax.fori_loop(0, n2 // 2, p2, 0)

    def fin(i, c):
        ocopy(i).wait()
        return c
    lax.fori_loop(0, n2, fin, 0)


@jax.jit
def pallas_sequential_preLN__linear_attn_block__glu_gated_reglu__prompt_kernel(A_x, A_wqkv, A_wo, B_x, B_W_gate, B_W_up, B_W_down):
    del B_x
    x = A_x.reshape(S, D)
    n1 = S // T1
    n2 = S // T2
    anyspec = pl.BlockSpec(memory_space=pl.ANY)
    out = pl.pallas_call(
        _kernel,
        out_shape=jax.ShapeDtypeStruct((S, D), BF),
        in_specs=[anyspec] * 6,
        out_specs=anyspec,
        scratch_shapes=[
            pltpu.VMEM((S, D), BF), pltpu.VMEM((S, D), BF),
            pltpu.VMEM((D, D), BF), pltpu.VMEM((D, D), BF), pltpu.VMEM((D, D), BF), pltpu.VMEM((D, D), BF), pltpu.VMEM((D, D), BF),
            pltpu.VMEM((D, D), BF), pltpu.VMEM((D, F), BF), pltpu.VMEM((D, F), BF), pltpu.VMEM((F, D), BF),
            pltpu.VMEM((S, D), BF), pltpu.VMEM((S, D), F32),
            pltpu.VMEM((D, D), F32), pltpu.VMEM((D, 128), F32), pltpu.VMEM((D, D), BF),
            pltpu.VMEM((NT, D, 128), F32), pltpu.VMEM((8, D), F32),
            pltpu.SemaphoreType.DMA((n1 + 9,)), pltpu.SemaphoreType.DMA((n2,)),
        ],
        compiler_params=pltpu.CompilerParams(vmem_limit_bytes=100 * 1024 * 1024),
    )(x, A_wqkv, A_wo, B_W_gate, B_W_up, B_W_down)
    return out.reshape(1, S, D)
```
